```python
import os as _os
_os.environ.setdefault("JAX_PLATFORMS", "cpu")
import jax
import jax.numpy as jnp

def _softmax(x, axis=-1):
    return jax.nn.softmax(x, axis=axis)
def _gelu(x):
    return jax.nn.gelu(x, approximate=True)
def _silu(x):
    return jax.nn.silu(x)
def _sigmoid(x):
    return jax.nn.sigmoid(x)
def _layernorm(x, axis=-1, eps=1e-5):
    m = jnp.mean(x, axis=axis, keepdims=True)
    v = jnp.var(x, axis=axis, keepdims=True)
    return (x - m) / jnp.sqrt(v + eps)
def _scatter_add(tgt, idx, src, axis=0):
    return tgt.at[idx].add(src)
def _segment_sum(src, seg, n):
    return jax.ops.segment_sum(src, seg, n)
class _Rng:
    def __init__(self, key):
        self._k = key
    def _next(self):
        self._k, sub = jax.random.split(self._k)
        return sub
    def normal(self, shape):
        return jax.random.normal(self._next(), shape, dtype=jnp.bfloat16)
    def randint(self, lo, hi, shape):
        return jax.random.randint(self._next(), shape, lo, hi, dtype=jnp.int32)
    def uniform(self, shape, lo=0.0, hi=1.0):
        return jax.random.uniform(self._next(), shape, jnp.bfloat16, lo, hi)
    def permutation(self, n):
        return jax.random.permutation(self._next(), n)


kernel_name = 'sequential_preLN__mha_block__swiglu_ffn__prompt'

def setup_inputs():
    _rng = _Rng(jax.random.key(int.from_bytes(__import__("os").urandom(4), "little")))
    _w = (lambda a: (lambda t: t.astype(jnp.bfloat16) if jnp.issubdtype(t.dtype, jnp.floating) else t)(jnp.asarray(a)))
    def _A_setup():
        B, S, D, H = 1, 2048, 640, 32
        return {
            "x": _w((lambda *s: _rng.normal(s) * 0.05)(B, S, D)),
            "wqkv": _w((lambda *s: _rng.normal(s) * 0.05)(D, 3 * D)),
            "wo": _w((lambda *s: _rng.normal(s) * 0.05)(D, D)),
        }
    _A_in = _A_setup()

    def _B_setup():
        B, S, D, F = 1, 2048, 640, 1728
        return {
            "x": _w((lambda *s: _rng.normal(s) * 0.05)(B, S, D)),
            "w_gate": _w((lambda *s: _rng.normal(s) * 0.05)(D, F)),
            "w_up": _w((lambda *s: _rng.normal(s) * 0.05)(D, F)),
            "w_down": _w((lambda *s: _rng.normal(s) * 0.05)(F, D)),
        }
    _B_in = _B_setup()

    return {
        "A_x": _A_in["x"],
        "A_wqkv": _A_in["wqkv"],
        "A_wo": _A_in["wo"],
        "B_x": _B_in["x"],
        "B_w_gate": _B_in["w_gate"],
        "B_w_up": _B_in["w_up"],
        "B_w_down": _B_in["w_down"],
    }

def reference(A_x, A_wqkv, A_wo, B_x, B_w_gate, B_w_up, B_w_down):
    def _A_ref(x, wqkv, wo):
        B, S, D = x.shape
        H = 32
        Dh = D // H
        qkv = (lambda x, *d: x.transpose(*d))((x @ wqkv).reshape(B, S, 3, H, Dh), 2, 0, 3, 1, 4)
        q, k, v = qkv[0], qkv[1], qkv[2]
        scores = jnp.einsum("bhqd,bhkd->bhqk", q, k) * (Dh ** -0.5)
        p = _softmax(scores, axis=-1)
        o = jnp.einsum("bhqk,bhkd->bhqd", p, v)
        return (lambda x, *d: x.transpose(*d))(o, 0, 2, 1, 3).reshape(B, S, D) @ wo

    def _B_ref(x, w_gate, w_up, w_down):
        g = _silu(x @ w_gate)
        u = x @ w_up
        return (g * u) @ w_down

    x = A_x
    h = x + _A_ref(_layernorm(x, axis=-1), A_wqkv, A_wo)
    h2 = h + _B_ref(_layernorm(h, axis=-1), B_w_gate, B_w_up, B_w_down)
    return h2
```

```python
import math

import jax
import jax.numpy as jnp
from jax import lax
import jax.experimental.pallas as pl
import jax.experimental.pallas.tpu as pltpu

S, D, H, DH, F = 2048, 640, 32, 20, 1728
EPS = 1e-5
F32 = jnp.float32
BF16 = jnp.bfloat16

TB = 512
NBB = S // TB
TQ = 512
NQ = S // TQ
KC = 128
NC = S // KC
TM = 256
NB = S // TM
F_CHUNKS = ((0, 512), (512, 512), (1024, 512), (1536, 128), (1664, 64))
NKB = D // 128 + 1

QSCALE = (DH ** -0.5) * math.log2(math.e)


def _head_geom(h):
    off = DH * h
    g0 = 16 * (off // 16)
    r0 = off - g0
    if off % 128 > 128 - DH:
        blk, dst = NKB - 1, 32 * (off // 128)
    else:
        blk = off // 128
        dst = g0 - 128 * blk
    ones_row = (r0 + DH) % 32
    return g0, r0, blk, dst, ones_row


def _layernorm(x):
    mu = jnp.sum(x, axis=-1, keepdims=True) * (1.0 / D)
    xc = x - mu
    var = jnp.sum(xc * xc, axis=-1, keepdims=True) * (1.0 / D)
    return xc * lax.rsqrt(var + EPS)


def _dot(a, b):
    return jnp.dot(a, b, preferred_element_type=F32)


def _dot_nt(a, b):
    return lax.dot_general(a, b, (((1,), (1,)), ((), ())), preferred_element_type=F32)


def _kernel(x_hbm, wqkv_hbm, wo_hbm, wgt_hbm, wut_hbm, wd_hbm, out_hbm,
            x_v, wqkv_v, wo_v, wgu_v, wd_v, wqt_v, wvt_v, xn_v,
            k_v, qtm_v, vt_v, s0_v, s1_v, s2_v, s3_v, m_v, ot_v,
            h_v, act_v, out_v, in_sem, out_sem):
    s_bufs = (s0_v, s1_v, s2_v, s3_v)

    x_cps = [pltpu.make_async_copy(x_hbm.at[pl.ds(i * TB, TB)],
                                   x_v.at[pl.ds(i * TB, TB)], in_sem.at[i])
             for i in range(NBB)]
    w_pairs = [(wqkv_hbm, wqkv_v), (wo_hbm, wo_v), (wd_hbm, wd_v)]
    for f0, fw in F_CHUNKS:
        w_pairs.append((wgt_hbm.at[pl.ds(f0, fw)], wgu_v.at[pl.ds(2 * f0, fw)]))
        w_pairs.append((wut_hbm.at[pl.ds(f0, fw)], wgu_v.at[pl.ds(2 * f0 + fw, fw)]))
    w_cps = [pltpu.make_async_copy(src, dst, in_sem.at[NBB + j])
             for j, (src, dst) in enumerate(w_pairs)]
    for cp in x_cps + w_cps:
        cp.start()

    def zero_body(h, c):
        qtm_v[h] = jnp.zeros((128, S), BF16)
        return c
    lax.fori_loop(0, H, zero_body, 0)

    for i in range(NBB):
        x_cps[i].wait()

        def ln1_body(j, c, i=i):
            r = pl.multiple_of(i * TB + j * 128, 128)
            xb = x_v[pl.ds(r, 128), :].astype(F32)
            xn_v[pl.ds(r, 128), :] = _layernorm(xb).astype(BF16)
            return c
        lax.fori_loop(0, TB // 128, ln1_body, 0)

    w_cps[0].wait()
    wqt_v[...] = wqkv_v[:, 0:D].T
    wvt_v[...] = wqkv_v[:, 2 * D:3 * D].T

    row32 = lax.broadcasted_iota(jnp.int32, (32, TB), 0)
    lane = lax.broadcasted_iota(jnp.int32, (TB, 128), 1)

    def qkv_body(i, c):
        r = pl.multiple_of(i * TB, TB)
        xb = xn_v[pl.ds(r, TB), :]
        vt = _dot_nt(wvt_v[...], xb)
        for h in range(H):
            g0, _, _, _, ones_row = _head_geom(h)
            win = jnp.where(row32 == ones_row, 1.0, vt[g0:g0 + 32, :])
            vt_v[h, :, pl.ds(r, TB)] = win.astype(BF16)
        qt = _dot_nt(wqt_v[...], xb) * QSCALE
        for h in range(H):
            g0, r0, _, dst, _ = _head_geom(h)
            keep = (row32 >= r0) & (row32 < r0 + DH)
            win = jnp.where(keep, qt[g0:g0 + 32, :], 0.0)
            qtm_v[h, dst:dst + 32, pl.ds(r, TB)] = win.astype(BF16)
        kf = _dot(xb, wqkv_v[:, D:2 * D])
        kb = [kf[:, 128 * b:128 * (b + 1)] for b in range(D // 128)]
        for b in range(D // 128):
            k_v[b, pl.ds(r, TB), :] = kb[b].astype(BF16)
        ext = None
        for b in range(4):
            comb = jnp.where(lane >= 112, kb[b], kb[b + 1])
            rolled = pltpu.roll(comb, 32 * b + 16, 1)
            ext = rolled if ext is None else jnp.where(lane >= 32 * b, rolled, ext)
        k_v[NKB - 1, pl.ds(r, TB), :] = ext.astype(BF16)
        return c
    lax.fori_loop(0, NBB, qkv_body, 0)

    def attn_step(h_cur, h_next):
        if h_next is not None:
            off = DH * h_next
            if isinstance(h_next, int):
                blk = _head_geom(h_next)[2]
            else:
                blk = jnp.where((off & 127) > 128 - DH, NKB - 1,
                                lax.shift_right_logical(off, 7))
        for j in range(NQ):
            s_ref = s_bufs[j]
            cols = slice(j * TQ, (j + 1) * TQ)
            if h_next is not None:
                w = qtm_v[h_next, :, cols]
            if h_cur is not None:
                m_cur = jnp.max(m_v[j], axis=0, keepdims=True)
            m = None
            acc = None
            for c in range(NC):
                rows = slice(c * KC, (c + 1) * KC)
                if h_cur is not None:
                    p = jnp.exp2(s_ref[rows, :] - m_cur).astype(BF16)
                if h_next is not None:
                    s = _dot(k_v[blk, rows, :], w)
                    s_ref[rows, :] = s
                    mc = jnp.max(s.reshape(KC // 8, 8, TQ), axis=0)
                    m = mc if m is None else jnp.maximum(m, mc)
                if h_cur is not None:
                    d = _dot(vt_v[h_cur, :, rows], p)
                    acc = d if acc is None else acc + d
            if h_cur is not None:
                ot_v[h_cur, :, cols] = acc
            if h_next is not None:
                m_v[j] = m

    attn_step(None, 0)

    def attn_body(h, c):
        attn_step(h, h + 1)
        return c
    lax.fori_loop(0, H - 1, attn_body, 0)
    attn_step(H - 1, None)

    for cp in w_cps[1:]:
        cp.wait()

    sub8 = lax.broadcasted_iota(jnp.int32, (8, TM), 0)

    def prep(r):
        tiles = []
        for k in range(H // 2):
            sc = []
            for h in (2 * k, 2 * k + 1):
                _, r0, _, _, ones_row = _head_geom(h)
                t0 = r0 // 8
                inv = 1.0 / ot_v[h, ones_row:ones_row + 1, pl.ds(r, TM)]
                sc.append(ot_v[h, 8 * t0:8 * t0 + 24, pl.ds(r, TM)] * inv)
            a, b = sc
            tiles += [a[0:16], jnp.where(sub8 < 4, a[16:24], b[0:8]), b[8:24]]
        o = jnp.concatenate(tiles, axis=0).T.astype(BF16)
        hh = x_v[pl.ds(r, TM), :].astype(F32) + _dot(o, wo_v[...])
        h_v[pl.ds(r, TM), :] = hh
        xn_v[pl.ds(r, TM), :] = _layernorm(hh).astype(BF16)

    def ffn_up(r):
        hn = xn_v[pl.ds(r, TM), :]
        for f0, fw in F_CHUNKS[:3]:
            gu = _dot_nt(hn, wgu_v[2 * f0:2 * (f0 + fw), :])
            g, u = gu[:, :fw], gu[:, fw:]
            act_v[:, f0:f0 + fw] = (g * jax.nn.sigmoid(g) * u).astype(BF16)
        gu = _dot_nt(hn, wgu_v[2 * F_CHUNKS[3][0]:, :])
        c0 = 0
        for f0, fw in F_CHUNKS[3:]:
            g, u = gu[:, c0:c0 + fw], gu[:, c0 + fw:c0 + 2 * fw]
            act_v[:, f0:f0 + fw] = (g * jax.nn.sigmoid(g) * u).astype(BF16)
            c0 += 2 * fw

    def out_copy(i, r):
        return pltpu.make_async_copy(out_v.at[pl.ds(r, TM)],
                                     out_hbm.at[pl.ds(r, TM)], out_sem.at[i])

    def ffn_down(i, r):
        y = _dot(act_v[...], wd_v[...])
        out_v[pl.ds(r, TM), :] = (h_v[pl.ds(r, TM), :] + y).astype(BF16)
        out_copy(i, r).start()

    prep(0)

    def ffn_body(i, c):
        r = pl.multiple_of(i * TM, TM)
        ffn_up(r)
        prep(pl.multiple_of(r + TM, TM))
        ffn_down(i, r)
        return c
    lax.fori_loop(0, NB - 1, ffn_body, 0)
    ffn_up((NB - 1) * TM)
    ffn_down(NB - 1, (NB - 1) * TM)

    for i in range(NB):
        out_copy(i, i * TM).wait()


@jax.jit
def pallas_sequential_preLN__mha_block__swiglu_ffn__prompt_kernel(
    A_x: jax.Array,
    A_wqkv: jax.Array,
    A_wo: jax.Array,
    B_x: jax.Array,
    B_w_gate: jax.Array,
    B_w_up: jax.Array,
    B_w_down: jax.Array,
):
    del B_x
    x2d = A_x.reshape(S, D)
    any_spec = pl.BlockSpec(memory_space=pltpu.HBM)
    out = pl.pallas_call(
        _kernel,
        in_specs=[any_spec] * 6,
        out_specs=any_spec,
        out_shape=jax.ShapeDtypeStruct((S, D), BF16),
        scratch_shapes=[
            pltpu.VMEM((S, D), BF16),
            pltpu.VMEM((D, 3 * D), BF16),
            pltpu.VMEM((D, D), BF16),
            pltpu.VMEM((2 * F, D), BF16),
            pltpu.VMEM((F, D), BF16),
            pltpu.VMEM((D, D), BF16),
            pltpu.VMEM((D, D), BF16),
            pltpu.VMEM((S, D), BF16),
            pltpu.VMEM((NKB, S, 128), BF16),
            pltpu.VMEM((H, 128, S), BF16),
            pltpu.VMEM((H, 32, S), BF16),
            pltpu.VMEM((S, TQ), F32),
            pltpu.VMEM((S, TQ), F32),
            pltpu.VMEM((S, TQ), F32),
            pltpu.VMEM((S, TQ), F32),
            pltpu.VMEM((NQ, 8, TQ), F32),
            pltpu.VMEM((H, 32, S), F32),
            pltpu.VMEM((S, D), F32),
            pltpu.VMEM((TM, F), BF16),
            pltpu.VMEM((S, D), BF16),
            pltpu.SemaphoreType.DMA((NBB + 3 + 2 * len(F_CHUNKS),)),
            pltpu.SemaphoreType.DMA((NB,)),
        ],
        compiler_params=pltpu.CompilerParams(vmem_limit_bytes=112 * 1024 * 1024),
    )(x2d, A_wqkv, A_wo, B_w_gate.T, B_w_up.T, B_w_down)
    return out.reshape(1, S, D)
```

```python
import math

import jax
import jax.numpy as jnp
from jax import lax
import jax.experimental.pallas as pl
import jax.experimental.pallas.tpu as pltpu

S, D, H, DH, F = 2048, 640, 32, 20, 1728
EPS = 1e-5
F32 = jnp.float32
BF16 = jnp.bfloat16

TB = 512
NBB = S // TB
TQ = 512
NQ = S // TQ
KC = 128
NC = S // KC
TM = 256
NB = S // TM
NFT = -(-F // 128)
UP_PIECES = ((10, 14), (0, 4), (4, 8), (8, 10))
PREP_AT = 3
N_SPLIT = 384
NKB = D // 128 + 1

QSCALE = (DH ** -0.5) * math.log2(math.e)


def _head_geom(h):
    off = DH * h
    g0 = 16 * (off // 16)
    r0 = off - g0
    if off % 128 > 128 - DH:
        blk, dst = NKB - 1, 32 * (off // 128)
    else:
        blk = off // 128
        dst = g0 - 128 * blk
    ones_row = (r0 + DH) % 32
    return g0, r0, blk, dst, ones_row


def _layernorm(x):
    mu = jnp.sum(x, axis=-1, keepdims=True) * (1.0 / D)
    xc = x - mu
    var = jnp.sum(xc * xc, axis=-1, keepdims=True) * (1.0 / D)
    return xc * lax.rsqrt(var + EPS)


def _dot(a, b):
    return jnp.dot(a, b, preferred_element_type=F32)


def _dot_nt(a, b):
    return lax.dot_general(a, b, (((1,), (1,)), ((), ())), preferred_element_type=F32)


def _kernel(x_hbm, wqkv_hbm, wo_hbm, wgt_hbm, wut_hbm, wd_hbm, out_hbm,
            x_v, wqkv_v, wo_v, wgu_v, wd_v, xn_v,
            k_v, qt_v, vt_v, s0_v, s1_v, s2_v, s3_v, m_v, ot_v,
            h_v, act_v, out_v, in_sem, out_sem):
    s_bufs = (s0_v, s1_v, s2_v, s3_v)

    def x_copy(i):
        r = i * TB if isinstance(i, int) else pl.multiple_of(i * TB, TB)
        return pltpu.make_async_copy(x_hbm.at[pl.ds(r, TB)],
                                     x_v.at[pl.ds(r, TB)], in_sem.at[i])
    w_pairs = [(wqkv_hbm.at[pl.ds(j * 160, 160)], wqkv_v.at[pl.ds(j * 160, 160)])
               for j in range(4)]
    w_cps = [pltpu.make_async_copy(src, dst, in_sem.at[NBB + j])
             for j, (src, dst) in enumerate(w_pairs)]
    late_pairs = [(wo_hbm, wo_v), (wd_hbm, wd_v)]
    for t in range(NFT):
        fw = min(128, F - 128 * t)
        late_pairs.append((wgt_hbm.at[pl.ds(128 * t, fw)],
                           wgu_v.at[pl.ds(256 * t, fw)]))
        late_pairs.append((wut_hbm.at[pl.ds(128 * t, fw)],
                           wgu_v.at[pl.ds(256 * t + fw, fw)]))
    late_cps = [pltpu.make_async_copy(src, dst, in_sem.at[NBB + 4])
                for src, dst in late_pairs]
    for cp in [x_copy(0)] + w_cps:
        cp.start()

    row32 = lax.broadcasted_iota(jnp.int32, (32, TB), 0)
    lane = lax.broadcasted_iota(jnp.int32, (TB, 128), 1)

    def ln1(r):
        for j in range(TB // 128):
            rows = pl.ds(r + j * 128, 128)
            xn_v[rows, :] = _layernorm(x_v[rows, :].astype(F32)).astype(BF16)

    def k_proj(rows):
        kf = _dot(xn_v[rows, :], wqkv_v[:, D:2 * D])
        kb = [kf[:, 128 * b:128 * (b + 1)] for b in range(D // 128)]
        for b in range(D // 128):
            k_v[b, rows, :] = kb[b].astype(BF16)
        ext = None
        for b in range(4):
            comb = jnp.where(lane >= 112, kb[b], kb[b + 1])
            rolled = pltpu.roll(comb, 32 * b + 16, 1)
            ext = rolled if ext is None else jnp.where(lane >= 32 * b, rolled, ext)
        k_v[NKB - 1, rows, :] = ext.astype(BF16)

    def v_proj(rows):
        vt = _dot_nt(wqkv_v[:, 2 * D:3 * D].T, xn_v[rows, :])
        for h in range(H):
            g0, _, _, _, ones_row = _head_geom(h)
            win = jnp.where(row32 == ones_row, 1.0, vt[g0:g0 + 32, :])
            vt_v[h, :, rows] = win.astype(BF16)

    def q_proj(rows):
        qt = _dot_nt(wqkv_v[:, 0:D].T, xn_v[rows, :]) * QSCALE
        for b in range(D // 128):
            qt_v[b, :, rows] = qt[128 * b:128 * (b + 1), :].astype(BF16)
        for b in range(4):
            qt_v[NKB - 1, 32 * b:32 * (b + 1), rows] = (
                qt[128 * b + 112:128 * b + 144, :].astype(BF16))

    x_copy(0).wait()
    x_copy(1).start()
    ln1(0)
    for cp in w_cps:
        cp.wait()
    for i in range(2, NBB):
        x_copy(i).start()

    def qkv_body(i, c):
        i_next = jnp.minimum(i + 1, NBB - 1)

        @pl.when(i + 1 < NBB)
        def _():
            x_copy(i_next).wait()
        rows = pl.ds(pl.multiple_of(i * TB, TB), TB)
        rn = pl.multiple_of(i_next * TB, TB)
        k_proj(rows)
        v_proj(rows)
        q_proj(rows)
        ln1(rn)
        return c
    lax.fori_loop(0, NBB, qkv_body, 0)

    row64 = lax.broadcasted_iota(jnp.int32, (64, TQ), 0)

    def head_sel(h_next):
        if isinstance(h_next, int):
            _, r0, blk, dst, _ = _head_geom(h_next)
            lo = dst + r0
        else:
            off = DH * h_next
            b = lax.shift_right_logical(off, 7)
            o = off & 127
            straddle = o > 128 - DH
            blk = jnp.where(straddle, NKB - 1, b)
            lo = jnp.where(straddle, 32 * b + o - 112, o)
        return blk, (2 * row64 >= lo) & (2 * row64 < lo + DH)

    def attn_stream(j, h_cur, sel):
        s_ref = s_bufs[j]
        cols = slice(j * TQ, (j + 1) * TQ)
        if sel is not None:
            blk, keep = sel
            w32 = pltpu.bitcast(qt_v[blk, :, cols], jnp.uint32)
            w = pltpu.bitcast(jnp.where(keep, w32, jnp.uint32(0)), BF16)
        if h_cur is not None:
            m_cur = jnp.max(m_v[j], axis=0, keepdims=True)
        m = None
        acc = None
        for c in range(NC):
            rows = slice(c * KC, (c + 1) * KC)
            if h_cur is not None:
                p = jnp.exp2(s_ref[rows, :] - m_cur).astype(BF16)
            if sel is not None:
                s = _dot(k_v[blk, rows, :], w)
                s_ref[rows, :] = s
                mc = jnp.max(s.reshape(KC // 8, 8, TQ), axis=0)
                m = mc if m is None else jnp.maximum(m, mc)
            if h_cur is not None:
                d = _dot(vt_v[h_cur, :, rows], p)
                acc = d if acc is None else acc + d
            if c == NC - 1:
                if h_cur is not None:
                    ot_v[h_cur, :, cols] = acc
                if sel is not None:
                    m_v[j] = m
            yield

    def attn_step(h_cur, h_next):
        sel = None if h_next is None else head_sel(h_next)
        for j in range(NQ):
            for _ in attn_stream(j, h_cur, sel):
                pass

    for cp in late_cps:
        cp.start()
    attn_step(None, 0)

    def attn_body(h, c):
        attn_step(h, h + 1)
        return c
    lax.fori_loop(0, H - 1, attn_body, 0)

    for cp in late_cps:
        cp.wait()

    sub8 = lax.broadcasted_iota(jnp.int32, (8, TM), 0)

    def prep(r):
        tiles = []
        for k in range(H // 2):
            sc = []
            for h in (2 * k, 2 * k + 1):
                _, r0, _, _, ones_row = _head_geom(h)
                t0 = r0 // 8
                inv = 1.0 / ot_v[h, ones_row:ones_row + 1, pl.ds(r, TM)]
                sc.append(ot_v[h, 8 * t0:8 * t0 + 24, pl.ds(r, TM)] * inv)
            a, b = sc
            tiles += [a[0:16], jnp.where(sub8 < 4, a[16:24], b[0:8]), b[8:24]]
        o = jnp.concatenate(tiles, axis=0).T.astype(BF16)
        hh = x_v[pl.ds(r, TM), :].astype(F32) + _dot(o, wo_v[...])
        h_v[pl.ds(r, TM), :] = hh
        xn_v[pl.ds(r, TM), :] = _layernorm(hh).astype(BF16)

    def ffn_up(r, t0, t1, m0=0, m1=TM):
        gu = _dot_nt(xn_v[pl.ds(r + m0, m1 - m0), :],
                     wgu_v[256 * t0:min(256 * t1, 2 * F), :])
        for t in range(t0, t1):
            fw = min(128, F - 128 * t)
            c0 = 256 * (t - t0)
            g, u = gu[:, c0:c0 + fw], gu[:, c0 + fw:c0 + 2 * fw]
            act_v[m0:m1, 128 * t:128 * t + fw] = (
                g * jax.nn.sigmoid(g) * u).astype(BF16)

    def ffn_down(r, n0, n1):
        y = _dot(act_v[...], wd_v[:, n0:n1])
        out_v[pl.ds(r, TM), n0:n1] = (h_v[pl.ds(r, TM), n0:n1] + y).astype(BF16)

    def out_copy(i, r):
        return pltpu.make_async_copy(out_v.at[pl.ds(r, TM)],
                                     out_hbm.at[pl.ds(r, TM)], out_sem.at[i])

    for _ in attn_stream(0, H - 1, None):
        pass
    for c, _ in enumerate(attn_stream(1, H - 1, None)):
        if c == PREP_AT:
            prep(0)
    n = 0
    for j in (2, 3):
        for c, _ in enumerate(attn_stream(j, H - 1, None)):
            if c % 4 == 1:
                ffn_up(0, n // 2, n // 2 + 1, (n % 2) * (TM // 2), (n % 2 + 1) * (TM // 2))
                n += 1
    t = n // 2
    ffn_up(0, 10, 14)
    ffn_up(0, t, 8)
    ffn_up(0, 8, 10)

    def ffn_body(i, c):
        r = pl.multiple_of(i * TM, TM)
        rn = pl.multiple_of(r + TM, TM)
        ffn_down(r, 0, N_SPLIT)
        prep(rn)
        ffn_down(r, N_SPLIT, D)
        out_copy(i, r).start()
        for t0, t1 in UP_PIECES:
            ffn_up(rn, t0, t1)
        return c
    lax.fori_loop(0, NB - 1, ffn_body, 0)
    ffn_down((NB - 1) * TM, 0, D)
    out_copy(NB - 1, (NB - 1) * TM).start()

    for i in range(NB):
        out_copy(i, i * TM).wait()


@jax.jit
def pallas_sequential_preLN__mha_block__swiglu_ffn__prompt_kernel(
    A_x: jax.Array,
    A_wqkv: jax.Array,
    A_wo: jax.Array,
    B_x: jax.Array,
    B_w_gate: jax.Array,
    B_w_up: jax.Array,
    B_w_down: jax.Array,
):
    del B_x
    x2d = A_x.reshape(S, D)
    any_spec = pl.BlockSpec(memory_space=pltpu.HBM)
    out = pl.pallas_call(
        _kernel,
        in_specs=[any_spec] * 6,
        out_specs=any_spec,
        out_shape=jax.ShapeDtypeStruct((S, D), BF16),
        scratch_shapes=[
            pltpu.VMEM((S, D), BF16),
            pltpu.VMEM((D, 3 * D), BF16),
            pltpu.VMEM((D, D), BF16),
            pltpu.VMEM((2 * F, D), BF16),
            pltpu.VMEM((F, D), BF16),
            pltpu.VMEM((S, D), BF16),
            pltpu.VMEM((NKB, S, 128), BF16),
            pltpu.VMEM((NKB, 128, S), BF16),
            pltpu.VMEM((H, 32, S), BF16),
            pltpu.VMEM((S, TQ), F32),
            pltpu.VMEM((S, TQ), F32),
            pltpu.VMEM((S, TQ), F32),
            pltpu.VMEM((S, TQ), F32),
            pltpu.VMEM((NQ, 8, TQ), F32),
            pltpu.VMEM((H, 32, S), F32),
            pltpu.VMEM((S, D), F32),
            pltpu.VMEM((TM, F), BF16),
            pltpu.VMEM((S, D), BF16),
            pltpu.SemaphoreType.DMA((NBB + 5,)),
            pltpu.SemaphoreType.DMA((NB,)),
        ],
        compiler_params=pltpu.CompilerParams(vmem_limit_bytes=100 * 1024 * 1024),
    )(x2d, A_wqkv, A_wo, B_w_gate.T, B_w_up.T, B_w_down)
    return out.reshape(1, S, D)
```

```python
import math

import jax
import jax.numpy as jnp
from jax import lax
import jax.experimental.pallas as pl
import jax.experimental.pallas.tpu as pltpu

S, D, H, DH, F = 2048, 640, 32, 20, 1728
EPS = 1e-5
F32 = jnp.float32
BF16 = jnp.bfloat16

TB = 512
NBB = S // TB
TH = TB // 2
TQ = 512
NQ = S // TQ
KC = 128
NC = S // KC
TM = 256
NB = S // TM
NFT = -(-F // 128)
UP_PIECES = ((10, 14), (0, 4), (4, 8), (8, 10))
PREP_AT = 3
N_SPLIT = 384
NKB = D // 128 + 1

QSCALE = (DH ** -0.5) * math.log2(math.e)


def _head_geom(h):
    off = DH * h
    g0 = 16 * (off // 16)
    r0 = off - g0
    if off % 128 > 128 - DH:
        blk, dst = NKB - 1, 32 * (off // 128)
    else:
        blk = off // 128
        dst = g0 - 128 * blk
    ones_row = (r0 + DH) % 32
    return g0, r0, blk, dst, ones_row


def _layernorm(x):
    mu = jnp.sum(x, axis=-1, keepdims=True) * (1.0 / D)
    xc = x - mu
    var = jnp.sum(xc * xc, axis=-1, keepdims=True) * (1.0 / D)
    return xc * lax.rsqrt(var + EPS)


def _dot(a, b):
    return jnp.dot(a, b, preferred_element_type=F32)


def _dot_nt(a, b):
    return lax.dot_general(a, b, (((1,), (1,)), ((), ())), preferred_element_type=F32)


def _kernel(x_hbm, wqkv_hbm, wo_hbm, wgt_hbm, wut_hbm, wd_hbm, out_hbm,
            x_v, wqkv_v, wo_v, wgu_v, wd_v, xn_v, xa_v, xb_v,
            k_v, qt_v, vt_v, s0_v, s1_v, s2_v, s3_v, m_v, ot_v,
            h_v, act_v, out_v, in_sem, out_sem):
    s_bufs = (s0_v, s1_v, s2_v, s3_v)

    def x_copy(i):
        r = i * TB if isinstance(i, int) else pl.multiple_of(i * TB, TB)
        return pltpu.make_async_copy(x_hbm.at[pl.ds(r, TB)],
                                     x_v.at[pl.ds(r, TB)], in_sem.at[i])
    w_pairs = [(wqkv_hbm.at[pl.ds(j * 160, 160)], wqkv_v.at[pl.ds(j * 160, 160)])
               for j in range(4)]
    w_cps = [pltpu.make_async_copy(src, dst, in_sem.at[NBB + j])
             for j, (src, dst) in enumerate(w_pairs)]
    late_pairs = [(wo_hbm, wo_v), (wd_hbm, wd_v)]
    for t in range(NFT):
        fw = min(128, F - 128 * t)
        late_pairs.append((wgt_hbm.at[pl.ds(128 * t, fw)],
                           wgu_v.at[pl.ds(256 * t, fw)]))
        late_pairs.append((wut_hbm.at[pl.ds(128 * t, fw)],
                           wgu_v.at[pl.ds(256 * t + fw, fw)]))
    late_cps = [pltpu.make_async_copy(src, dst, in_sem.at[NBB + 4])
                for src, dst in late_pairs]
    for cp in [x_copy(0)] + w_cps:
        cp.start()

    row32 = lax.broadcasted_iota(jnp.int32, (32, TH), 0)
    lane = lax.broadcasted_iota(jnp.int32, (TH, 128), 1)

    def ln1(r, dst):
        for j in range(TH // 128):
            xb = x_v[pl.ds(r + j * 128, 128), :].astype(F32)
            dst[j * 128:(j + 1) * 128, :] = _layernorm(xb).astype(BF16)

    def qkv_proj(src, rows, wqt, wvt):
        kf = _dot(src[...], wqkv_v[:, D:2 * D])
        kb = [kf[:, 128 * b:128 * (b + 1)] for b in range(D // 128)]
        for b in range(D // 128):
            k_v[b, rows, :] = kb[b].astype(BF16)
        ext = None
        for b in range(4):
            comb = jnp.where(lane >= 112, kb[b], kb[b + 1])
            rolled = pltpu.roll(comb, 32 * b + 16, 1)
            ext = rolled if ext is None else jnp.where(lane >= 32 * b, rolled, ext)
        k_v[NKB - 1, rows, :] = ext.astype(BF16)
        vt = _dot_nt(wvt, src[...])
        for h in range(H):
            g0, _, _, _, ones_row = _head_geom(h)
            win = jnp.where(row32 == ones_row, 1.0, vt[g0:g0 + 32, :])
            vt_v[h, :, rows] = win.astype(BF16)
        qt = _dot_nt(wqt, src[...]) * QSCALE
        for b in range(D // 128):
            qt_v[b, :, rows] = qt[128 * b:128 * (b + 1), :].astype(BF16)
        for b in range(4):
            qt_v[NKB - 1, 32 * b:32 * (b + 1), rows] = (
                qt[128 * b + 112:128 * b + 144, :].astype(BF16))

    x_copy(0).wait()
    x_copy(1).start()
    ln1(0, xa_v)
    for cp in w_cps:
        cp.wait()
    for i in range(2, NBB):
        x_copy(i).start()

    def qkv_body(i, c):
        i_next = jnp.minimum(i + 1, NBB - 1)

        @pl.when(i + 1 < NBB)
        def _():
            x_copy(i_next).wait()
        r = pl.multiple_of(i * TB, TB)
        wvt = wqkv_v[:, 2 * D:3 * D].T
        wqt = wqkv_v[:, 0:D].T
        ln1(r + TH, xb_v)
        qkv_proj(xa_v, pl.ds(r, TH), wqt, wvt)
        qkv_proj(xb_v, pl.ds(pl.multiple_of(r + TH, TH), TH), wqt, wvt)
        ln1(pl.multiple_of(i_next * TB, TB), xa_v)
        return c
    lax.fori_loop(0, NBB, qkv_body, 0)

    row64 = lax.broadcasted_iota(jnp.int32, (64, TQ), 0)

    def head_sel(h_next):
        if isinstance(h_next, int):
            _, r0, blk, dst, _ = _head_geom(h_next)
            lo = dst + r0
        else:
            off = DH * h_next
            b = lax.shift_right_logical(off, 7)
            o = off & 127
            straddle = o > 128 - DH
            blk = jnp.where(straddle, NKB - 1, b)
            lo = jnp.where(straddle, 32 * b + o - 112, o)
        return blk, (2 * row64 >= lo) & (2 * row64 < lo + DH)

    def attn_stream(j, h_cur, sel):
        s_ref = s_bufs[j]
        cols = slice(j * TQ, (j + 1) * TQ)
        if sel is not None:
            blk, keep = sel
            w32 = pltpu.bitcast(qt_v[blk, :, cols], jnp.uint32)
            w = pltpu.bitcast(jnp.where(keep, w32, jnp.uint32(0)), BF16)
        if h_cur is not None:
            m_cur = jnp.max(m_v[j], axis=0, keepdims=True)
        m = None
        acc = None
        for c in range(NC):
            rows = slice(c * KC, (c + 1) * KC)
            if h_cur is not None:
                p = jnp.exp2(s_ref[rows, :] - m_cur).astype(BF16)
            if sel is not None:
                s = _dot(k_v[blk, rows, :], w)
                s_ref[rows, :] = s
                mc = jnp.max(s.reshape(KC // 8, 8, TQ), axis=0)
                m = mc if m is None else jnp.maximum(m, mc)
            if h_cur is not None:
                d = _dot(vt_v[h_cur, :, rows], p)
                acc = d if acc is None else acc + d
            if c == NC - 1:
                if h_cur is not None:
                    ot_v[h_cur, :, cols] = acc
                if sel is not None:
                    m_v[j] = m
            yield

    def attn_step(h_cur, h_next):
        sel = None if h_next is None else head_sel(h_next)
        for j in range(NQ):
            for _ in attn_stream(j, h_cur, sel):
                pass

    for cp in late_cps:
        cp.start()
    attn_step(None, 0)

    def attn_body(h, c):
        attn_step(h, h + 1)
        return c
    lax.fori_loop(0, H - 1, attn_body, 0)

    for cp in late_cps:
        cp.wait()

    sub8 = lax.broadcasted_iota(jnp.int32, (8, TM), 0)

    def prep(r):
        tiles = []
        for k in range(H // 2):
            sc = []
            for h in (2 * k, 2 * k + 1):
                _, r0, _, _, ones_row = _head_geom(h)
                t0 = r0 // 8
                inv = 1.0 / ot_v[h, ones_row:ones_row + 1, pl.ds(r, TM)]
                sc.append(ot_v[h, 8 * t0:8 * t0 + 24, pl.ds(r, TM)] * inv)
            a, b = sc
            tiles += [a[0:16], jnp.where(sub8 < 4, a[16:24], b[0:8]), b[8:24]]
        o = jnp.concatenate(tiles, axis=0).T.astype(BF16)
        hh = x_v[pl.ds(r, TM), :].astype(F32) + _dot(o, wo_v[...])
        h_v[pl.ds(r, TM), :] = hh
        xn_v[pl.ds(r, TM), :] = _layernorm(hh).astype(BF16)

    def ffn_up(r, t0, t1, m0=0, m1=TM):
        gu = _dot_nt(xn_v[pl.ds(r + m0, m1 - m0), :],
                     wgu_v[256 * t0:min(256 * t1, 2 * F), :])
        for t in range(t0, t1):
            fw = min(128, F - 128 * t)
            c0 = 256 * (t - t0)
            g, u = gu[:, c0:c0 + fw], gu[:, c0 + fw:c0 + 2 * fw]
            act_v[m0:m1, 128 * t:128 * t + fw] = (
                g * jax.nn.sigmoid(g) * u).astype(BF16)

    def ffn_down(r, n0, n1):
        y = _dot(act_v[...], wd_v[:, n0:n1])
        out_v[pl.ds(r, TM), n0:n1] = (h_v[pl.ds(r, TM), n0:n1] + y).astype(BF16)

    def out_copy(i, r):
        return pltpu.make_async_copy(out_v.at[pl.ds(r, TM)],
                                     out_hbm.at[pl.ds(r, TM)], out_sem.at[i])

    for _ in attn_stream(0, H - 1, None):
        pass
    for c, _ in enumerate(attn_stream(1, H - 1, None)):
        if c == PREP_AT:
            prep(0)
    n = 0
    for j in (2, 3):
        for c, _ in enumerate(attn_stream(j, H - 1, None)):
            if c % 4 == 1:
                ffn_up(0, n // 2, n // 2 + 1, (n % 2) * (TM // 2), (n % 2 + 1) * (TM // 2))
                n += 1
    t = n // 2
    ffn_up(0, 10, 14)
    ffn_up(0, t, 8)
    ffn_up(0, 8, 10)

    def ffn_body(i, c):
        r = pl.multiple_of(i * TM, TM)
        rn = pl.multiple_of(r + TM, TM)
        ffn_down(r, 0, N_SPLIT)
        prep(rn)
        ffn_down(r, N_SPLIT, D)
        out_copy(i, r).start()
        for t0, t1 in UP_PIECES:
            ffn_up(rn, t0, t1)
        return c
    lax.fori_loop(0, NB - 1, ffn_body, 0)
    ffn_down((NB - 1) * TM, 0, D)
    out_copy(NB - 1, (NB - 1) * TM).start()

    for i in range(NB):
        out_copy(i, i * TM).wait()


@jax.jit
def pallas_sequential_preLN__mha_block__swiglu_ffn__prompt_kernel(
    A_x: jax.Array,
    A_wqkv: jax.Array,
    A_wo: jax.Array,
    B_x: jax.Array,
    B_w_gate: jax.Array,
    B_w_up: jax.Array,
    B_w_down: jax.Array,
):
    del B_x
    x2d = A_x.reshape(S, D)
    any_spec = pl.BlockSpec(memory_space=pltpu.HBM)
    out = pl.pallas_call(
        _kernel,
        in_specs=[any_spec] * 6,
        out_specs=any_spec,
        out_shape=jax.ShapeDtypeStruct((S, D), BF16),
        scratch_shapes=[
            pltpu.VMEM((S, D), BF16),
            pltpu.VMEM((D, 3 * D), BF16),
            pltpu.VMEM((D, D), BF16),
            pltpu.VMEM((2 * F, D), BF16),
            pltpu.VMEM((F, D), BF16),
            pltpu.VMEM((S, D), BF16),
            pltpu.VMEM((TH, D), BF16),
            pltpu.VMEM((TH, D), BF16),
            pltpu.VMEM((NKB, S, 128), BF16),
            pltpu.VMEM((NKB, 128, S), BF16),
            pltpu.VMEM((H, 32, S), BF16),
            pltpu.VMEM((S, TQ), F32),
            pltpu.VMEM((S, TQ), F32),
            pltpu.VMEM((S, TQ), F32),
            pltpu.VMEM((S, TQ), F32),
            pltpu.VMEM((NQ, 8, TQ), F32),
            pltpu.VMEM((H, 32, S), F32),
            pltpu.VMEM((S, D), F32),
            pltpu.VMEM((TM, F), BF16),
            pltpu.VMEM((S, D), BF16),
            pltpu.SemaphoreType.DMA((NBB + 5,)),
            pltpu.SemaphoreType.DMA((NB,)),
        ],
        compiler_params=pltpu.CompilerParams(vmem_limit_bytes=100 * 1024 * 1024),
    )(x2d, A_wqkv, A_wo, B_w_gate.T, B_w_up.T, B_w_down)
    return out.reshape(1, S, D)
```

```python
import math

import jax
import jax.numpy as jnp
from jax import lax
import jax.experimental.pallas as pl
import jax.experimental.pallas.tpu as pltpu

S, D, H, DH, F = 2048, 640, 32, 20, 1728
EPS = 1e-5
F32 = jnp.float32
BF16 = jnp.bfloat16

TB = 512
NBB = S // TB
TH = TB // 2
NXH = S // TH
TQ = 512
NQ = S // TQ
KC = 128
NC = S // KC
TM = 256
NB = S // TM
NFT = -(-F // 128)
UP_PIECES = ((10, 14), (0, 4), (4, 8), (8, 10))
PREP_AT = 3
N_SPLIT = 384
NKB = D // 128 + 1

QSCALE = (DH ** -0.5) * math.log2(math.e)


def _head_geom(h):
    off = DH * h
    g0 = 16 * (off // 16)
    r0 = off - g0
    if off % 128 > 128 - DH:
        blk, dst = NKB - 1, 32 * (off // 128)
    else:
        blk = off // 128
        dst = g0 - 128 * blk
    ones_row = (r0 + DH) % 32
    return g0, r0, blk, dst, ones_row


def _layernorm(x):
    mu = jnp.sum(x, axis=-1, keepdims=True) * (1.0 / D)
    xc = x - mu
    var = jnp.sum(xc * xc, axis=-1, keepdims=True) * (1.0 / D)
    return xc * lax.rsqrt(var + EPS)


def _dot(a, b):
    return jnp.dot(a, b, preferred_element_type=F32)


def _dot_nt(a, b):
    return lax.dot_general(a, b, (((1,), (1,)), ((), ())), preferred_element_type=F32)


def _kernel(x_hbm, wqkv_hbm, wo_hbm, wgt_hbm, wut_hbm, wd_hbm, out_hbm,
            x_v, wqkv_v, wo_v, wgu_v, wd_v, xn_v, xa_v, xb_v,
            k_v, qt_v, vt_v, s0_v, s1_v, s2_v, s3_v, m_v, ot_v,
            h_v, act_v, out_v, in_sem, out_sem):
    s_bufs = (s0_v, s1_v, s2_v, s3_v)

    def x_copy(i):
        r = i * TH if isinstance(i, int) else pl.multiple_of(i * TH, TH)
        return pltpu.make_async_copy(x_hbm.at[pl.ds(r, TH)],
                                     x_v.at[pl.ds(r, TH)], in_sem.at[i])
    w_pairs = [(wqkv_hbm.at[pl.ds(j * 160, 160)], wqkv_v.at[pl.ds(j * 160, 160)])
               for j in range(4)]
    w_cps = [pltpu.make_async_copy(src, dst, in_sem.at[NXH + j])
             for j, (src, dst) in enumerate(w_pairs)]
    late_pairs = [(wo_hbm, wo_v), (wd_hbm, wd_v)]
    for t in range(NFT):
        fw = min(128, F - 128 * t)
        late_pairs.append((wgt_hbm.at[pl.ds(128 * t, fw)],
                           wgu_v.at[pl.ds(256 * t, fw)]))
        late_pairs.append((wut_hbm.at[pl.ds(128 * t, fw)],
                           wgu_v.at[pl.ds(256 * t + fw, fw)]))
    late_cps = [pltpu.make_async_copy(src, dst, in_sem.at[NXH + 4])
                for src, dst in late_pairs]
    for cp in [x_copy(0)] + w_cps:
        cp.start()

    row32 = lax.broadcasted_iota(jnp.int32, (32, TH), 0)
    lane = lax.broadcasted_iota(jnp.int32, (TH, 128), 1)

    def ln1(r, dst):
        for j in range(TH // 128):
            xb = x_v[pl.ds(r + j * 128, 128), :].astype(F32)
            dst[j * 128:(j + 1) * 128, :] = _layernorm(xb).astype(BF16)

    def qkv_proj(src, rows, wqt, wvt):
        kf = _dot(src[...], wqkv_v[:, D:2 * D])
        kb = [kf[:, 128 * b:128 * (b + 1)] for b in range(D // 128)]
        for b in range(D // 128):
            k_v[b, rows, :] = kb[b].astype(BF16)
        ext = None
        for b in range(4):
            comb = jnp.where(lane >= 112, kb[b], kb[b + 1])
            rolled = pltpu.roll(comb, 32 * b + 16, 1)
            ext = rolled if ext is None else jnp.where(lane >= 32 * b, rolled, ext)
        k_v[NKB - 1, rows, :] = ext.astype(BF16)
        vt = _dot_nt(wvt, src[...])
        for h in range(H):
            g0, _, _, _, ones_row = _head_geom(h)
            win = jnp.where(row32 == ones_row, 1.0, vt[g0:g0 + 32, :])
            vt_v[h, :, rows] = win.astype(BF16)
        qt = _dot_nt(wqt, src[...]) * QSCALE
        for b in range(D // 128):
            qt_v[b, :, rows] = qt[128 * b:128 * (b + 1), :].astype(BF16)
        for b in range(4):
            qt_v[NKB - 1, 32 * b:32 * (b + 1), rows] = (
                qt[128 * b + 112:128 * b + 144, :].astype(BF16))

    x_copy(0).wait()
    x_copy(1).start()
    x_copy(2).start()
    ln1(0, xa_v)
    for cp in w_cps:
        cp.wait()
    for i in range(3, NXH):
        x_copy(i).start()

    def qkv_body(i, c):
        i_next = jnp.minimum(i + 1, NBB - 1)
        x_copy(2 * i + 1).wait()

        @pl.when(i + 1 < NBB)
        def _():
            x_copy(2 * i_next).wait()
        r = pl.multiple_of(i * TB, TB)
        wvt = wqkv_v[:, 2 * D:3 * D].T
        wqt = wqkv_v[:, 0:D].T
        ln1(r + TH, xb_v)
        qkv_proj(xa_v, pl.ds(r, TH), wqt, wvt)
        qkv_proj(xb_v, pl.ds(pl.multiple_of(r + TH, TH), TH), wqt, wvt)
        ln1(pl.multiple_of(i_next * TB, TB), xa_v)
        return c
    lax.fori_loop(0, NBB, qkv_body, 0)

    row64 = lax.broadcasted_iota(jnp.int32, (64, TQ), 0)

    def head_sel(h_next):
        if isinstance(h_next, int):
            _, r0, blk, dst, _ = _head_geom(h_next)
            lo = dst + r0
        else:
            off = DH * h_next
            b = lax.shift_right_logical(off, 7)
            o = off & 127
            straddle = o > 128 - DH
            blk = jnp.where(straddle, NKB - 1, b)
            lo = jnp.where(straddle, 32 * b + o - 112, o)
        return blk, (2 * row64 >= lo) & (2 * row64 < lo + DH)

    def attn_stream(j, h_cur, sel):
        s_ref = s_bufs[j]
        cols = slice(j * TQ, (j + 1) * TQ)
        if sel is not None:
            blk, keep = sel
            w32 = pltpu.bitcast(qt_v[blk, :, cols], jnp.uint32)
            w = pltpu.bitcast(jnp.where(keep, w32, jnp.uint32(0)), BF16)
        if h_cur is not None:
            m_cur = jnp.max(m_v[j], axis=0, keepdims=True)
        m = None
        acc = None
        for c in range(NC):
            rows = slice(c * KC, (c + 1) * KC)
            if h_cur is not None:
                p = jnp.exp2(s_ref[rows, :] - m_cur).astype(BF16)
            if sel is not None:
                s = _dot(k_v[blk, rows, :], w)
                s_ref[rows, :] = s
                mc = jnp.max(s.reshape(KC // 8, 8, TQ), axis=0)
                m = mc if m is None else jnp.maximum(m, mc)
            if h_cur is not None:
                d = _dot(vt_v[h_cur, :, rows], p)
                acc = d if acc is None else acc + d
            if c == NC - 1:
                if h_cur is not None:
                    ot_v[h_cur, :, cols] = acc
                if sel is not None:
                    m_v[j] = m
            yield

    def attn_step(h_cur, h_next):
        sel = None if h_next is None else head_sel(h_next)
        for j in range(NQ):
            for _ in attn_stream(j, h_cur, sel):
                pass

    for cp in late_cps:
        cp.start()
    attn_step(None, 0)

    def attn_body(h, c):
        attn_step(h, h + 1)
        return c
    lax.fori_loop(0, H - 1, attn_body, 0)

    for cp in late_cps:
        cp.wait()

    sub8 = lax.broadcasted_iota(jnp.int32, (8, TM), 0)

    def prep(r):
        tiles = []
        for k in range(H // 2):
            sc = []
            for h in (2 * k, 2 * k + 1):
                _, r0, _, _, ones_row = _head_geom(h)
                t0 = r0 // 8
                inv = 1.0 / ot_v[h, ones_row:ones_row + 1, pl.ds(r, TM)]
                sc.append(ot_v[h, 8 * t0:8 * t0 + 24, pl.ds(r, TM)] * inv)
            a, b = sc
            tiles += [a[0:16], jnp.where(sub8 < 4, a[16:24], b[0:8]), b[8:24]]
        o = jnp.concatenate(tiles, axis=0).T.astype(BF16)
        hh = x_v[pl.ds(r, TM), :].astype(F32) + _dot(o, wo_v[...])
        h_v[pl.ds(r, TM), :] = hh
        xn_v[pl.ds(r, TM), :] = _layernorm(hh).astype(BF16)

    def ffn_up(r, t0, t1, m0=0, m1=TM):
        gu = _dot_nt(xn_v[pl.ds(r + m0, m1 - m0), :],
                     wgu_v[256 * t0:min(256 * t1, 2 * F), :])
        for t in range(t0, t1):
            fw = min(128, F - 128 * t)
            c0 = 256 * (t - t0)
            g, u = gu[:, c0:c0 + fw], gu[:, c0 + fw:c0 + 2 * fw]
            act_v[m0:m1, 128 * t:128 * t + fw] = (
                g * jax.nn.sigmoid(g) * u).astype(BF16)

    def ffn_down(r, n0, n1):
        y = _dot(act_v[...], wd_v[:, n0:n1])
        out_v[pl.ds(r, TM), n0:n1] = (h_v[pl.ds(r, TM), n0:n1] + y).astype(BF16)

    def out_copy(i, r):
        return pltpu.make_async_copy(out_v.at[pl.ds(r, TM)],
                                     out_hbm.at[pl.ds(r, TM)], out_sem.at[i])

    for _ in attn_stream(0, H - 1, None):
        pass
    for c, _ in enumerate(attn_stream(1, H - 1, None)):
        if c == PREP_AT:
            prep(0)
    n = 0
    for j in (2, 3):
        for c, _ in enumerate(attn_stream(j, H - 1, None)):
            if c % 4 == 1:
                ffn_up(0, n // 2, n // 2 + 1, (n % 2) * (TM // 2), (n % 2 + 1) * (TM // 2))
                n += 1
    t = n // 2
    ffn_up(0, 10, 14)
    ffn_up(0, t, 8)
    ffn_up(0, 8, 10)

    def ffn_body(i, c):
        r = pl.multiple_of(i * TM, TM)
        rn = pl.multiple_of(r + TM, TM)
        ffn_down(r, 0, N_SPLIT)
        prep(rn)
        ffn_down(r, N_SPLIT, D)
        out_copy(i, r).start()
        for t0, t1 in UP_PIECES:
            ffn_up(rn, t0, t1)
        return c
    lax.fori_loop(0, NB - 1, ffn_body, 0)
    ffn_down((NB - 1) * TM, 0, D)
    out_copy(NB - 1, (NB - 1) * TM).start()

    for i in range(NB):
        out_copy(i, i * TM).wait()


@jax.jit
def pallas_sequential_preLN__mha_block__swiglu_ffn__prompt_kernel(
    A_x: jax.Array,
    A_wqkv: jax.Array,
    A_wo: jax.Array,
    B_x: jax.Array,
    B_w_gate: jax.Array,
    B_w_up: jax.Array,
    B_w_down: jax.Array,
):
    del B_x
    x2d = A_x.reshape(S, D)
    any_spec = pl.BlockSpec(memory_space=pltpu.HBM)
    out = pl.pallas_call(
        _kernel,
        in_specs=[any_spec] * 6,
        out_specs=any_spec,
        out_shape=jax.ShapeDtypeStruct((S, D), BF16),
        scratch_shapes=[
            pltpu.VMEM((S, D), BF16),
            pltpu.VMEM((D, 3 * D), BF16),
            pltpu.VMEM((D, D), BF16),
            pltpu.VMEM((2 * F, D), BF16),
            pltpu.VMEM((F, D), BF16),
            pltpu.VMEM((S, D), BF16),
            pltpu.VMEM((TH, D), BF16),
            pltpu.VMEM((TH, D), BF16),
            pltpu.VMEM((NKB, S, 128), BF16),
            pltpu.VMEM((NKB, 128, S), BF16),
            pltpu.VMEM((H, 32, S), BF16),
            pltpu.VMEM((S, TQ), F32),
            pltpu.VMEM((S, TQ), F32),
            pltpu.VMEM((S, TQ), F32),
            pltpu.VMEM((S, TQ), F32),
            pltpu.VMEM((NQ, 8, TQ), F32),
            pltpu.VMEM((H, 32, S), F32),
            pltpu.VMEM((S, D), F32),
            pltpu.VMEM((TM, F), BF16),
            pltpu.VMEM((S, D), BF16),
            pltpu.SemaphoreType.DMA((NXH + 5,)),
            pltpu.SemaphoreType.DMA((NB,)),
        ],
        compiler_params=pltpu.CompilerParams(vmem_limit_bytes=100 * 1024 * 1024),
    )(x2d, A_wqkv, A_wo, B_w_gate.T, B_w_up.T, B_w_down)
    return out.reshape(1, S, D)
```
